```python
import os as _os
_os.environ.setdefault("JAX_PLATFORMS", "cpu")
import jax
import jax.numpy as jnp

def _softmax(x, axis=-1):
    return jax.nn.softmax(x, axis=axis)
def _gelu(x):
    return jax.nn.gelu(x, approximate=True)
def _silu(x):
    return jax.nn.silu(x)
def _sigmoid(x):
    return jax.nn.sigmoid(x)
def _layernorm(x, axis=-1, eps=1e-5):
    m = jnp.mean(x, axis=axis, keepdims=True)
    v = jnp.var(x, axis=axis, keepdims=True)
    return (x - m) / jnp.sqrt(v + eps)
def _scatter_add(tgt, idx, src, axis=0):
    return tgt.at[idx].add(src)
def _segment_sum(src, seg, n):
    return jax.ops.segment_sum(src, seg, n)
class _Rng:
    def __init__(self, key):
        self._k = key
    def _next(self):
        self._k, sub = jax.random.split(self._k)
        return sub
    def normal(self, shape):
        return jax.random.normal(self._next(), shape, dtype=jnp.bfloat16)
    def randint(self, lo, hi, shape):
        return jax.random.randint(self._next(), shape, lo, hi, dtype=jnp.int32)
    def uniform(self, shape, lo=0.0, hi=1.0):
        return jax.random.uniform(self._next(), shape, jnp.bfloat16, lo, hi)
    def permutation(self, n):
        return jax.random.permutation(self._next(), n)


kernel_name = 'standalone__channel_attn_cbam__vision'

def setup_inputs():
    _rng = _Rng(jax.random.key(int.from_bytes(__import__("os").urandom(4), "little")))
    _w = (lambda a: (lambda t: t.astype(jnp.bfloat16) if jnp.issubdtype(t.dtype, jnp.floating) else t)(jnp.asarray(a)))
    H = W = 224
    C = 192
    r = max(C // 4, 1)
    return {
        "x": _w((lambda *s: _rng.normal(s) * 0.2)(1, H, W, C) + (lambda *s: _rng.normal(s) * 0.2)(1, 1, 1, C) * 2.0),
        "w1": _w((lambda *s: _rng.normal(s) * 0.2)(C, r)),
        "w2": _w((lambda *s: _rng.normal(s) * 0.2)(r, C)),
    }

def reference(x, w1, w2):
    B, H, W, C = x.shape
    xf = x.reshape(B, H * W, C)
    gap = jnp.mean(xf, 1)
    gmp = jnp.amax(xf, 1)
    h_a = gap @ w1
    h_a = h_a * (lambda x, dt: x.astype(dt))(h_a > 0, h_a.dtype)
    h_m = gmp @ w1
    h_m = h_m * (lambda x, dt: x.astype(dt))(h_m > 0, h_m.dtype)
    scale = _sigmoid(h_a @ w2 + h_m @ w2)
    return x * scale[:, None, None, :]
```

```python
import jax
import jax.numpy as jnp
from jax import lax
import jax.experimental.pallas as pl
import jax.experimental.pallas.tpu as pltpu

F32 = jnp.float32
BF16 = jnp.bfloat16

A = 7
CB = 32
LAST_ROWS = (20, 8, 3, 1)
K = 1
UNROLL = 16


def _round_bf16(v):
    return v.astype(BF16).astype(F32)


def _cbam_kernel(x_hbm, w1t_hbm, w2_hbm, o_hbm,
                 buf, w1t_v, w2_v, w1c_v, w2c_v, scale_v, out_sem):
    _, HH, C, W = x_hbm.shape
    R = w1t_v.shape[0]
    n_pix = A * HH * W
    nb = C // CB

    plan = [(j, 0, A, 0, HH) for j in range(nb - 1)]
    plan += [(nb - 1, 0, A - 3, 0, HH), (nb - 1, A - 3, 2, 0, HH)]
    h0 = 0
    for n in LAST_ROWS:
        plan.append((nb - 1, A - 1, 1, h0, n))
        h0 += n
    assert h0 == HH
    n_in = len(plan)

    def body(sems):
        def window(ref, p):
            j, a0, na, hh0, nh = p
            cs = pl.ds(j * CB, CB)
            if nh == HH:
                return ref.at[pl.ds(a0, na), :, cs]
            return ref.at[a0, pl.ds(hh0, nh), cs]

        def in_copy(i):
            return pltpu.make_async_copy(
                window(x_hbm, plan[i]), window(buf, plan[i]), sems.at[i])

        w1_copy = pltpu.make_async_copy(w1t_hbm, w1t_v, sems.at[n_in])
        w2_copy = pltpu.make_async_copy(w2_hbm, w2_v, sems.at[n_in + 1])
        w1_copy.start()
        w2_copy.start()
        for i in range(n_in):
            in_copy(i).start()
        w1_copy.wait()
        w2_copy.wait()
        w1c_v[...] = w1t_v[...].astype(F32).T
        w2c_v[...] = w2_v[...].astype(F32).T

        ha8 = jnp.zeros((8, R), F32)
        hm8 = jnp.zeros((8, R), F32)
        s = m = None
        for i, (j, a0, na, hh0, nh) in enumerate(plan):
            cs = pl.ds(j * CB, CB)
            in_copy(i).wait()
            if a0 == 0 and hh0 == 0:
                s = jnp.zeros((CB, W), F32)
                m = jnp.full((CB, W), -jnp.inf, F32)
            if nh == HH:
                per = HH // UNROLL

                def p1_body(t, carry, a0=a0, cs=cs, per=per):
                    s, m = carry
                    a = a0 + t // per
                    hb = (t % per) * UNROLL
                    for h in range(UNROLL):
                        v = buf[a, hb + h, cs, :].astype(F32)
                        s = s + v
                        m = jnp.maximum(m, v)
                    return s, m

                s, m = lax.fori_loop(0, na * per, p1_body, (s, m))
            else:
                for h in range(nh):
                    v = buf[a0, hh0 + h, cs, :].astype(F32)
                    s = s + v
                    m = jnp.maximum(m, v)
            if a0 + na == A and hh0 + nh == HH:
                gap = _round_bf16(jnp.sum(s, axis=1, keepdims=True) * (1.0 / n_pix))
                gmp = jnp.max(m, axis=1, keepdims=True)
                w1b = w1c_v[cs, :]
                pa = w1b * gap
                pm = w1b * gmp
                for k in range(CB // 8):
                    ha8 = ha8 + pa[8 * k:8 * k + 8]
                    hm8 = hm8 + pm[8 * k:8 * k + 8]

        ha = _round_bf16(jnp.sum(ha8, axis=0, keepdims=True))
        hm = _round_bf16(jnp.sum(hm8, axis=0, keepdims=True))
        ha = jnp.where(ha > 0, ha, 0.0)
        hm = jnp.where(hm > 0, hm, 0.0)

        def scale_block(c0):
            w2b = w2c_v[pl.ds(c0, CB), :]
            la = _round_bf16(jnp.sum(w2b * ha, axis=1, keepdims=True))
            lm = _round_bf16(jnp.sum(w2b * hm, axis=1, keepdims=True))
            sc = _round_bf16(jax.nn.sigmoid(_round_bf16(la + lm)))
            return jnp.broadcast_to(sc, (CB, 128))

        def p2_step(hh, c0, sc):
            cs = pl.ds(c0, CB)
            scw = jnp.concatenate([sc, sc[:, :W - 128]], axis=1)
            for a in range(A):
                v = buf[a, hh, cs, :].astype(F32)
                buf[a, hh, cs, :] = (v * scw).astype(BF16)
            pltpu.make_async_copy(
                buf.at[:, hh, cs], o_hbm.at[:, hh, cs], out_sem).start()

        def first_rows(c0):
            sc = scale_block(c0)
            for hh in range(K):
                p2_step(hh, c0, sc)
            scale_v[pl.ds(c0, CB), :] = sc

        first_rows(0)

        def blk_body(i, carry):
            first_rows(pl.multiple_of(i * CB, CB))
            return carry

        lax.fori_loop(1, nb, blk_body, 0)

        def p2_body(hh, carry):
            for j in range(nb):
                p2_step(hh, j * CB, scale_v[pl.ds(j * CB, CB), :])
            return carry

        lax.fori_loop(K, HH, p2_body, 0)

    pl.run_scoped(body, pltpu.SemaphoreType.DMA((n_in + 2,)))
    pltpu.make_async_copy(buf, o_hbm, out_sem).wait()


@jax.jit
def pallas_standalone__channel_attn_cbam__vision_kernel(
    x: jax.Array,
    w1: jax.Array,
    w2: jax.Array,
):
    B, H, W, C = x.shape
    R = w1.shape[1]
    assert B == 1 and H % A == 0 and C % CB == 0 and 128 < W <= 256
    HH = H // A
    xt = jnp.transpose(x, (0, 1, 3, 2)).reshape(A, HH, C, W)
    out = pl.pallas_call(
        _cbam_kernel,
        out_shape=jax.ShapeDtypeStruct((A, HH, C, W), x.dtype),
        in_specs=[pl.BlockSpec(memory_space=pl.ANY)] * 3,
        out_specs=pl.BlockSpec(memory_space=pl.ANY),
        scratch_shapes=[
            pltpu.VMEM((A, HH, C, W), x.dtype),
            pltpu.VMEM((R, C), w1.dtype),
            pltpu.VMEM((R, C), w2.dtype),
            pltpu.VMEM((C, R), F32),
            pltpu.VMEM((C, R), F32),
            pltpu.VMEM((C, 128), F32),
            pltpu.SemaphoreType.DMA(()),
        ],
        compiler_params=pltpu.CompilerParams(vmem_limit_bytes=48 * 1024 * 1024),
    )(xt, w1.T, w2)
    return jnp.transpose(out.reshape(B, H, C, W), (0, 1, 3, 2))
```

```python
import jax
import jax.numpy as jnp
from jax import lax
import jax.experimental.pallas as pl
import jax.experimental.pallas.tpu as pltpu

F32 = jnp.float32
BF16 = jnp.bfloat16

A = 7
CB = 24
TAIL = 16
LAST_ROWS = (10, 4, 1, 1)
HEAD = (8, 16)
OUT_BLOCKS = (24, 64, 56, 48)
UNROLL = 16


def _round_bf16(v):
    return v.astype(BF16).astype(F32)


def _relu(v):
    return v * (v > 0).astype(v.dtype)


def _cbam_kernel(x_hbm, w1t_hbm, w2_hbm, o_hbm,
                 buf, w1t_v, w2_v, w1c_v, w2c_v, acc_s, acc_m, scale_v):
    _, HH, C, W = x_hbm.shape
    R = w1t_v.shape[0]
    n_pix = A * HH * W
    nb = C // CB
    t0 = HH - TAIL

    main = [(0, A - 3, 0, HH), (A - 3, 1, 0, HH), (A - 2, 1, 0, HH), (A - 1, 1, 0, t0)]
    tail = [(j * CB, t0, TAIL) for j in range(nb - 1)]
    h0 = t0
    for n in LAST_ROWS:
        tail.append(((nb - 1) * CB, h0, n))
        h0 += n
    assert h0 == HH and sum(HEAD) == CB and sum(OUT_BLOCKS) == C
    n_main = len(main)
    n_in = n_main + len(tail)

    def body(sems, out_sem):
        def window(ref, i):
            if i < n_main:
                a0, na, hh0, nh = main[i]
                if nh == HH:
                    return ref.at[pl.ds(a0, na)]
                return ref.at[a0, pl.ds(hh0, nh)]
            c0, hh0, nh = tail[i - n_main]
            return ref.at[A - 1, pl.ds(hh0, nh), pl.ds(c0, CB)]

        def in_copy(i):
            return pltpu.make_async_copy(window(x_hbm, i), window(buf, i), sems.at[i])

        w1_copy = pltpu.make_async_copy(w1t_hbm, w1t_v, sems.at[n_in])
        w2_copy = pltpu.make_async_copy(w2_hbm, w2_v, sems.at[n_in + 1])
        w1_copy.start()
        w2_copy.start()
        for i in range(n_in):
            in_copy(i).start()
        w1_copy.wait()
        w2_copy.wait()
        w1c_v[...] = w1t_v[...].astype(F32).T
        w2c_v[...] = w2_v[...].astype(F32).T
        acc_s[...] = jnp.zeros(acc_s.shape, F32)
        acc_m[...] = jnp.full(acc_m.shape, -jnp.inf, F32)

        for i, (a0, na, hh0, nh) in enumerate(main):
            in_copy(i).wait()
            per = nh // UNROLL
            assert per * UNROLL == nh

            def p1_body(t, carry, a0=a0, hh0=hh0, per=per):
                g = t // nb
                a = a0 + g // per
                hb = hh0 + (g % per) * UNROLL
                cs = pl.ds(pl.multiple_of((t % nb) * CB, CB), CB)
                s = acc_s[cs, :]
                m = acc_m[cs, :]
                for h in range(UNROLL):
                    v = buf[a, hb + h, cs, :].astype(F32)
                    s = s + v
                    m = jnp.maximum(m, v)
                acc_s[cs, :] = s
                acc_m[cs, :] = m
                return carry

            lax.fori_loop(0, na * per * nb, p1_body, 0)

        ha8 = jnp.zeros((8, R), F32)
        hm8 = jnp.zeros((8, R), F32)
        s = m = None
        for i, (c0, hh0, nh) in enumerate(tail):
            cs = pl.ds(c0, CB)
            if hh0 == t0:
                s = acc_s[cs, :]
                m = acc_m[cs, :]
            in_copy(n_main + i).wait()
            for h in range(nh):
                v = buf[A - 1, hh0 + h, cs, :].astype(F32)
                s = s + v
                m = jnp.maximum(m, v)
            if hh0 + nh == HH:
                gap = _round_bf16(jnp.sum(s, axis=1, keepdims=True) * (1.0 / n_pix))
                gmp = jnp.max(m, axis=1, keepdims=True)
                w1b = w1c_v[cs, :]
                pa = w1b * gap
                pm = w1b * gmp
                for k in range(CB // 8):
                    ha8 = ha8 + pa[8 * k:8 * k + 8]
                    hm8 = hm8 + pm[8 * k:8 * k + 8]

        ha = _relu(_round_bf16(jnp.sum(ha8, axis=0, keepdims=True)))
        hm = _relu(_round_bf16(jnp.sum(hm8, axis=0, keepdims=True)))

        def logits(c0, cb):
            w2b = w2c_v[pl.ds(c0, cb), :]
            la = _round_bf16(jnp.sum(w2b * ha, axis=1, keepdims=True))
            lm = _round_bf16(jnp.sum(w2b * hm, axis=1, keepdims=True))
            return jnp.broadcast_to(_round_bf16(la + lm), (cb, 128))

        def p2_step(hh, c0, cb, sc):
            cs = pl.ds(c0, cb)
            scw = jnp.concatenate([sc, sc[:, :W - 128]], axis=1)
            for a in range(A):
                v = buf[a, hh, cs, :].astype(F32)
                buf[a, hh, cs, :] = (v * scw).astype(BF16)
            pltpu.make_async_copy(buf.at[:, hh, cs], o_hbm.at[:, hh, cs], out_sem).start()

        def first_row(c0, cb, lg):
            sc = _round_bf16(jax.nn.sigmoid(lg))
            p2_step(0, c0, cb, sc)
            scale_v[pl.ds(c0, cb), :] = sc

        head_off = [sum(HEAD[:k]) for k in range(len(HEAD))]
        head_lg = [logits(c0, cb) for c0, cb in zip(head_off, HEAD)]
        lg1 = logits(CB, CB)
        for c0, cb, lg in zip(head_off, HEAD, head_lg):
            first_row(c0, cb, lg)

        def blk_body(i, lg):
            nxt = jnp.minimum(i + 1, nb - 1)
            lg_next = logits(pl.multiple_of(nxt * CB, CB), CB)
            first_row(pl.multiple_of(i * CB, CB), CB, lg)
            return lg_next

        lax.fori_loop(1, nb, blk_body, lg1)

        def p2_body(hh, carry):
            c0 = 0
            for cb in OUT_BLOCKS:
                p2_step(hh, c0, cb, scale_v[pl.ds(c0, cb), :])
                c0 += cb
            return carry

        lax.fori_loop(1, HH, p2_body, 0)

        pltpu.make_async_copy(buf, o_hbm, out_sem).wait()

    pl.run_scoped(body, pltpu.SemaphoreType.DMA((n_in + 2,)), pltpu.SemaphoreType.DMA(()))


@jax.jit
def pallas_standalone__channel_attn_cbam__vision_kernel(
    x: jax.Array,
    w1: jax.Array,
    w2: jax.Array,
):
    B, H, W, C = x.shape
    R = w1.shape[1]
    assert B == 1 and H % A == 0 and C % CB == 0 and 128 < W <= 256
    HH = H // A
    xt = jnp.transpose(x, (0, 1, 3, 2)).reshape(A, HH, C, W)
    out = pl.pallas_call(
        _cbam_kernel,
        out_shape=jax.ShapeDtypeStruct((A, HH, C, W), x.dtype),
        in_specs=[pl.BlockSpec(memory_space=pl.ANY)] * 3,
        out_specs=pl.BlockSpec(memory_space=pl.ANY),
        scratch_shapes=[
            pltpu.VMEM((A, HH, C, W), x.dtype),
            pltpu.VMEM((R, C), w1.dtype),
            pltpu.VMEM((R, C), w2.dtype),
            pltpu.VMEM((C, R), F32),
            pltpu.VMEM((C, R), F32),
            pltpu.VMEM((C, W), F32),
            pltpu.VMEM((C, W), F32),
            pltpu.VMEM((C, 128), F32),
        ],
        compiler_params=pltpu.CompilerParams(vmem_limit_bytes=48 * 1024 * 1024),
    )(xt, w1.T, w2)
    return jnp.transpose(out.reshape(B, H, C, W), (0, 1, 3, 2))
```
